```python
import jax
import jax.numpy as jnp

def _softmax(x, axis=-1):
    return jax.nn.softmax(x, axis=axis)
def _gelu(x):
    return jax.nn.gelu(x, approximate=True)
def _silu(x):
    return jax.nn.silu(x)
def _sigmoid(x):
    return jax.nn.sigmoid(x)
def _layernorm(x, axis=-1, eps=1e-5):
    m = jnp.mean(x, axis=axis, keepdims=True)
    v = jnp.var(x, axis=axis, keepdims=True)
    return (x - m) / jnp.sqrt(v + eps)
def _scatter_add(tgt, idx, src, axis=0):
    return tgt.at[idx].add(src)
def _segment_sum(src, seg, n):
    return jax.ops.segment_sum(src, seg, n)
class _Rng:
    def __init__(self, key):
        self._k = key
    def _next(self):
        self._k, sub = jax.random.split(self._k)
        return sub
    def normal(self, shape):
        return jax.random.normal(self._next(), shape, dtype=jnp.bfloat16)
    def randint(self, lo, hi, shape):
        return jax.random.randint(self._next(), shape, lo, hi, dtype=jnp.int32)
    def uniform(self, shape, lo=0.0, hi=1.0):
        return jax.random.uniform(self._next(), shape, jnp.bfloat16, lo, hi)
    def permutation(self, n):
        return jax.random.permutation(self._next(), n)


kernel_name = 'interleave_layers__sliding_local_dilated__glu_gated_geglu__prompt'

def setup_inputs():
    _rng = _Rng(jax.random.key(int.from_bytes(__import__("os").urandom(4), "little")))
    _w = (lambda a: (lambda t: t.astype(jnp.bfloat16) if jnp.issubdtype(t.dtype, jnp.floating) else t)(jnp.asarray(a)))
    def _A_setup():
        B, S, D = 1, 2048, 576
        return {
            "x": _w((lambda *s: _rng.normal(s) * 0.05)(B, S, D)),
            "wqkv": _w((lambda *s: _rng.normal(s) * 0.05)(D, 3 * D)),
            "wo": _w((lambda *s: _rng.normal(s) * 0.05)(D, D)),
        }
    _A_in = _A_setup()

    def _B_setup():
        B, S, Dm, Df = 1, 2048, 576, 4608
        return {
            "x": _w((lambda *s: _rng.normal(s) * 0.05)(B, S, Dm)),
            "w_gate": _w((lambda *s: _rng.normal(s) * 0.05)(Dm, Df) * (Dm ** -0.5)),
            "w_up": _w((lambda *s: _rng.normal(s) * 0.05)(Dm, Df) * (Dm ** -0.5)),
            "w_down": _w((lambda *s: _rng.normal(s) * 0.05)(Df, Dm) * (Df ** -0.5)),
        }
    _B_in = _B_setup()

    return {
        "A_x": _A_in["x"],
        "A_wqkv": _A_in["wqkv"],
        "A_wo": _A_in["wo"],
        "B_x": _B_in["x"],
        "B_w_gate": _B_in["w_gate"],
        "B_w_up": _B_in["w_up"],
        "B_w_down": _B_in["w_down"],
    }

def reference(A_x, A_wqkv, A_wo, B_x, B_w_gate, B_w_up, B_w_down):
    def _A_ref(x, wqkv, wo):
        B, S, D = x.shape
        H = 32; Dh = D // H
        W, dil = 8, 2
        qkv = (lambda x, *d: x.transpose(*d))((x @ wqkv).reshape(B, S, 3, H, Dh), 2, 0, 3, 1, 4)
        q, k, v = qkv[0], qkv[1], qkv[2]
        scale = Dh ** -0.5
        pos = jnp.arange(S)
        off = jnp.arange(W) * dil
        idx = pos[:, None] - off[None, :]
        mask = idx >= 0
        idx_c = jnp.where(mask, idx, 0).reshape(-1)
        kg = k[:, :, idx_c, :].reshape(B, H, S, W, Dh)
        vg = v[:, :, idx_c, :].reshape(B, H, S, W, Dh)
        logits = jnp.einsum("bhsd,bhswd->bhsw", q, kg) * scale
        logits = jnp.where(mask[None, None, :, :], logits, -1e9)
        attn = _softmax(logits, axis=-1)
        o = jnp.einsum("bhsw,bhswd->bhsd", attn, vg)
        return (lambda x, *d: x.transpose(*d))(o, 0, 2, 1, 3).reshape(B, S, D) @ wo

    def _B_ref(x, w_gate, w_up, w_down):
        g = jnp.einsum("bsd,df->bsf", x, w_gate)
        u = jnp.einsum("bsd,df->bsf", x, w_up)
        h = _gelu(g) * u
        return jnp.einsum("bsf,fd->bsd", h, w_down)

    x = A_x
    x = x + _A_ref(_layernorm(x, axis=-1), A_wqkv, A_wo)
    x = x + _B_ref(_layernorm(x, axis=-1), B_w_gate, B_w_up, B_w_down)
    x = x + _A_ref(_layernorm(x, axis=-1), A_wqkv, A_wo)
    x = x + _B_ref(_layernorm(x, axis=-1), B_w_gate, B_w_up, B_w_down)
    return x
```

```python
import functools
import numpy as np
import jax
import jax.numpy as jnp
from jax import lax
import jax.experimental.pallas as pl
import jax.experimental.pallas.tpu as pltpu

S, D, H, DH, W, DIL, DF = 2048, 576, 32, 18, 8, 2, 4608
DP = 640
NQ = 1792
R = 256
NB = S // R
FC = 1152
NC = DF // FC
G = 128
f32, bf16 = jnp.float32, jnp.bfloat16
NT = (((1,), (1,)), ((), ()))
NN = (((1,), (0,)), ((), ()))


def _gelu(g):
    c = np.float32(np.sqrt(2.0 / np.pi))
    return 0.5 * g * (1.0 + jnp.tanh(c * (g + np.float32(0.044715) * (g * g * g))))


def kernel(xT_hbm, wqkv_hbm, wo_hbm, wg_hbm, wu_hbm, wdT_hbm, outT_hbm,
           xio, xs, wqkv_raw, wo_raw, wt, wall, woT, wg, wu, wdT, xn, xn_cur, xn_next, flag, xa, x1b, q_s, k_s, v_s, ksh, vsh, o_s, h_s, acc, sems):
    cp_x = pltpu.make_async_copy(xT_hbm, xio, sems.at[0])
    cp_qkv = pltpu.make_async_copy(wqkv_hbm, wqkv_raw, sems.at[1])
    cp_wo = pltpu.make_async_copy(wo_hbm, wo_raw, sems.at[2])
    def cp_ffn(c):
        sl = pl.ds(c * FC, FC)
        return [pltpu.make_async_copy(wg_hbm.at[:, sl], wg.at[pl.ds(0, D), sl], sems.at[3 + 3 * c]),
                pltpu.make_async_copy(wu_hbm.at[:, sl], wu.at[pl.ds(0, D), sl], sems.at[4 + 3 * c]),
                pltpu.make_async_copy(wdT_hbm.at[:, sl], wdT.at[:, sl], sems.at[5 + 3 * c])]
    cp_qkv.start()
    cp_x.start()
    cp_wo.start()
    cp_qkv.wait()
    for c_ in range(NC):
        for cp in cp_ffn(c_):
            cp.start()

    wg[D:DP, :] = jnp.zeros((DP - D, DF), bf16)
    wu[D:DP, :] = jnp.zeros((DP - D, DF), bf16)
    wall[...] = jnp.zeros(wall.shape, bf16)
    woT[...] = jnp.zeros(woT.shape, bf16)
    xn[...] = jnp.zeros(xn.shape, bf16)
    xn_cur[...] = jnp.zeros(xn_cur.shape, bf16)
    xn_next[...] = jnp.zeros(xn_next.shape, bf16)
    flag[...] = jnp.zeros(flag.shape, jnp.int32)
    wt[4] = jnp.zeros((3 * D, 128), f32)

    LW = [128, 128, 128, 128, 64]
    for t in range(0, 3 * D, 576):
        tr = wqkv_raw[:, t:t + 576].astype(f32).T
        for lt in range(5):
            wt[lt, t:t + 576, 0:LW[lt]] = tr[:, lt * 128:lt * 128 + LW[lt]]
    for p in range(3):
        for d in range(DH):
            if d < 16:
                base = p * 512 + d * 32
            else:
                base = 1536 + p * 64 + (d - 16) * 32
            for lt in range(5):
                blk = wt[lt, pl.ds(p * D + d, H, stride=DH), :]
                wall[base:base + H, lt * 128:lt * 128 + LW[lt]] = blk[:, 0:LW[lt]].astype(bf16)
    cp_wo.wait()
    wof = wo_raw[...].astype(f32)
    for lt in range(5):
        wt[lt, 0:D, 0:LW[lt]] = wof[:, lt * 128:lt * 128 + LW[lt]]
    rows = [jnp.concatenate([wt[lt, pl.ds(d, H, stride=DH), :][:, 0:LW[lt]] for lt in range(5)], axis=1) for d in range(DH)]
    wop = jnp.concatenate(rows, axis=0)
    woT[:, 0:D] = wop.T.astype(bf16)

    cp_x.wait()
    lane_full = lax.broadcasted_iota(jnp.int32, (D, 128), 1)
    perm_in = (lane_full % 8) * 16 + lane_full // 8
    perm_out = (lane_full % 16) * 8 + lane_full // 16
    for t_ in range(S // 128):
        xs[:, t_ * 128:(t_ + 1) * 128] = jnp.take_along_axis(xio[:, t_ * 128:(t_ + 1) * 128].astype(f32), perm_in, axis=1)

    scale = np.float32(DH ** -0.5)
    lane = lax.broadcasted_iota(jnp.int32, (8, 128), 1)
    lo = lane < 64

    def stage_ln(c0, dst):
        if c0 is None:
            xb = x1b[...]
        else:
            xb = xs[:, pl.ds(c0, R)]
            xa[...] = xb
        m = jnp.mean(xb, axis=0, keepdims=True)
        xc = xb - m
        v = jnp.mean(xc * xc, axis=0, keepdims=True)
        xnt = xc * (1.0 / jnp.sqrt(v + 1e-5))
        dst[:, 0:D] = xnt.T.astype(bf16)

    def stage_q(c0):
        xnv = xn[...]
        r1 = G
        q_s[:, 0:512] = lax.dot_general(xnv, wall[0:512, :], NT, preferred_element_type=f32)
        k_s[r1:r1 + R, 0:512] = lax.dot_general(xnv, wall[512:1024, :], NT, preferred_element_type=f32)
        v_s[r1:r1 + R, 0:512] = lax.dot_general(xnv, wall[1024:1536, :], NT, preferred_element_type=f32)
        tl = lax.dot_general(xnv, wall[1536:1792, :], NT, preferred_element_type=f32)
        lo_ = lax.broadcasted_iota(jnp.int32, (R, 128), 1) < 64
        t12 = tl[:, 0:128]
        q_s[:, 512:640] = jnp.where(lo_, t12, 0.0)
        k_s[r1:r1 + R, 512:640] = jnp.where(lo_, pltpu.roll(t12, 64, 1), 0.0)
        v_s[r1:r1 + R, 512:640] = tl[:, 128:256]

    sub = lax.broadcasted_iota(jnp.int32, (8, 128), 0)

    def t_shift(c0, g, tps):
        for tp in tps:
            rp = g * G + 8 * tp
            rc = (g + 1) * G + 8 * tp
            for tt in range(5):
                ls = slice(tt * 128, (tt + 1) * 128)
                ksh[g, tp - 2, :, ls] = pltpu.roll(jnp.where(sub == 7, k_s[rp:rp + 8, ls], k_s[rc:rc + 8, ls]), 1, 0)
                vsh[g, tp - 2, :, ls] = pltpu.roll(jnp.where(sub == 7, v_s[rp:rp + 8, ls], v_s[rc:rc + 8, ls]), 1, 0)

    def t_slab(c0, first, g, t, tok=None):
        def kv(buf, sh, w, ls):
            tau = t - w * DIL
            if tau >= 0:
                r0_ = (g + 1) * G + 8 * tau
                return buf[r0_:r0_ + 8, ls]
            return sh[g, tau + 16 - 2, :, ls]
        s0 = g * G + 8 * t
        q = [q_s[s0:s0 + 8, tt * 128:(tt + 1) * 128] for tt in range(5)]
        logits = []
        for w in range(W):
            tsum = None
            for tt in range(5):
                pr = q[tt] * kv(k_s, ksh, w, slice(tt * 128, (tt + 1) * 128))
                tsum = pr if tsum is None else tsum + pr
            if w == 0 and tok is not None:
                tsum = tsum + tok
            tsum = tsum + pltpu.roll(tsum, 64, 1)
            tsum = tsum + pltpu.roll(tsum, 32, 1)
            tsum = tsum * scale
            if g == 0 and t < w * DIL:
                bad = jnp.logical_and(first, sub == 0)
                tsum = jnp.where(bad, np.float32(-1e9), tsum)
            logits.append(tsum)
        m = logits[0]
        for w in range(1, W):
            m = jnp.maximum(m, logits[w])
        es = [jnp.exp(l - m) for l in logits]
        ssum = es[0]
        for w in range(1, W):
            ssum = ssum + es[w]
        inv = 1.0 / ssum
        for tt in range(5):
            ls = slice(tt * 128, (tt + 1) * 128)
            o = None
            for w in range(W):
                pv = es[w] * kv(v_s, vsh, w, ls)
                o = pv if o is None else o + pv
            o_s[s0:s0 + 8, ls] = o * inv

    def t_pieces(c0, first):
        P = functools.partial
        pcs = []
        for g in range(R // G):
            pcs.append(P(t_shift, c0, g, range(2, 9)))
            pcs.append(P(t_shift, c0, g, range(9, 16)))
            for t in range(15, -1, -1):
                pcs.append(P(t_slab, c0, first, g, t))
        return pcs

    def stage_t(c0, first):
        for p in t_pieces(c0, first):
            p()

    def stage_o(c0):
        y = lax.dot_general(woT[...], o_s[...].astype(bf16), NT, preferred_element_type=f32)
        x1b[...] = xa[...] + y
        k_s[0:G, :] = k_s[R:R + G, :]
        v_s[0:G, :] = v_s[R:R + G, :]

    NS = FC // 128

    def f_sub(c, sb, slot):
        f0 = c * FC + sb * 128
        xnv = xn_cur[...]
        g = jnp.dot(xnv, wg[:, f0:f0 + 128], preferred_element_type=f32)
        u = jnp.dot(xnv, wu[:, f0:f0 + 128], preferred_element_type=f32)
        h_s[c % 2, :, sb * 128:(sb + 1) * 128] = (_gelu(g) * u).astype(bf16)
        return g[0:8, :]

    def f_down(c):
        f0 = c * FC
        src = x1b if c == 0 else acc
        acc[...] = src[...] + lax.dot_general(wdT[:, f0:f0 + FC], h_s[c % 2], NT, preferred_element_type=f32)

    def halo_reset():
        k_s[0:G, :] = jnp.zeros((G, DP), f32)
        v_s[0:G, :] = jnp.zeros((G, DP), f32)

    def a_stage(piece, t):
        c0 = pl.multiple_of((t % NB) * R, R)
        if piece == 0:
            stage_ln(c0, xn)
        elif piece == 1:
            stage_q(c0)
        elif piece == 2:
            stage_t(c0, t % NB == 0)
        elif piece == 3:
            stage_o(c0)
            stage_ln(None, xn_cur)

    def slot(t, with_a):
        P = functools.partial
        c0 = pl.multiple_of((t % NB) * R, R)
        never = flag[...] != 0
        extra = {}
        if with_a:
            ca = pl.multiple_of(((t + 1) % NB) * R, R)
            first = (t + 1) % NB == 0
            extra[(0, 0)] = [lambda tok: stage_ln(ca, xn)]
            extra[(0, 3)] = [lambda tok: stage_q(ca)]
            extra[(0, 8)] = [lambda tok, g=g: t_shift(ca, g, range(2, 16)) for g in range(R // G)]
            tp = [(g, tt_) for g in range(R // G) for tt_ in range(15, -1, -1)]
            slots_ = [(1, i) for i in range(NS)] + [(2, i) for i in range(NS - 2)]
            for i, (g, tt_) in enumerate(tp):
                extra.setdefault(slots_[(i * len(slots_)) // len(tp)], []).append(
                    lambda tok, g=g, tt_=tt_: t_slab(ca, first, g, tt_, tok))
            extra[(2, NS - 1)] = [lambda tok: stage_o(ca), lambda tok: stage_ln(None, xn_next)]
        for c in range(NC):
            if c == 2 and with_a:
                @pl.when(t == 0)
                def _():
                    for c_ in range(2, 4):
                        for cp in cp_ffn(c_):
                            cp.wait()
            for sb in range(NS):
                dep = f_sub(c, sb, t % 2)
                if c > 0 and sb == 1:
                    f_down(c - 1)
                if (c, sb) in extra:
                    tok = jnp.where(never, dep, 0.0)
                    for p in extra[(c, sb)]:
                        p(tok)
        if with_a:
            xn_cur[...] = xn_next[...]
        f_down(NC - 1)
        xs[:, pl.ds(c0, R)] = acc[...]

    halo_reset()
    for p in range(4):
        a_stage(p, 0)
    for c_ in range(2):
        for cp in cp_ffn(c_):
            cp.wait()

    def body(t, carry):
        slot(t, True)
        return carry

    lax.fori_loop(0, 2 * NB - 1, body, 0)
    tl_ = 2 * NB - 1
    c0l = (tl_ % NB) * R
    acc[...] = x1b[...]

    def cbody(c, carry):
        f0 = pl.multiple_of(c * FC, FC)
        xnv = xn_cur[...]
        g = jnp.dot(xnv, wg[:, pl.ds(f0, FC)], preferred_element_type=f32)
        u = jnp.dot(xnv, wu[:, pl.ds(f0, FC)], preferred_element_type=f32)
        h = (_gelu(g) * u).astype(bf16)
        acc[...] += lax.dot_general(wdT[:, pl.ds(f0, FC)], h, NT, preferred_element_type=f32)
        return carry

    lax.fori_loop(0, NC, cbody, 0)
    xs[:, pl.ds(c0l, R)] = acc[...]
    for t_ in range(S // 128):
        xio[:, t_ * 128:(t_ + 1) * 128] = jnp.take_along_axis(xs[:, t_ * 128:(t_ + 1) * 128], perm_out, axis=1).astype(bf16)
    cp_o = pltpu.make_async_copy(xio, outT_hbm, sems.at[0])
    cp_o.start()
    cp_o.wait()


@jax.jit
def pallas_interleave_layers__sliding_local_dilated__glu_gated_geglu__prompt_kernel(
    A_x, A_wqkv, A_wo, B_x, B_w_gate, B_w_up, B_w_down):
    hbm = pl.BlockSpec(memory_space=pltpu.HBM)
    out = pl.pallas_call(
        kernel,
        out_shape=jax.ShapeDtypeStruct((D, S), bf16),
        in_specs=[hbm] * 6,
        out_specs=hbm,
        scratch_shapes=[
            pltpu.VMEM((D, S), bf16),
            pltpu.VMEM((D, S), f32),
            pltpu.VMEM((D, 3 * D), bf16),
            pltpu.VMEM((D, D), bf16),
            pltpu.VMEM((5, 3 * D, 128), f32),
            pltpu.VMEM((NQ, DP), bf16),
            pltpu.VMEM((D, DP), bf16),
            pltpu.VMEM((DP, DF), bf16),
            pltpu.VMEM((DP, DF), bf16),
            pltpu.VMEM((D, DF), bf16),
            pltpu.VMEM((R, DP), bf16),
            pltpu.VMEM((R, DP), bf16),
            pltpu.VMEM((R, DP), bf16),
            pltpu.VMEM((8, 128), jnp.int32),
            pltpu.VMEM((D, R), f32),
            pltpu.VMEM((D, R), f32),
            pltpu.VMEM((R, DP), f32),
            pltpu.VMEM((G + R, DP), f32),
            pltpu.VMEM((G + R, DP), f32),
            pltpu.VMEM((R // G, 14, 8, DP), f32),
            pltpu.VMEM((R // G, 14, 8, DP), f32),
            pltpu.VMEM((R, DP), f32),
            pltpu.VMEM((2, R, FC), bf16),
            pltpu.VMEM((D, R), f32),
            pltpu.SemaphoreType.DMA((3 + 3 * NC,)),
        ],
        compiler_params=pltpu.CompilerParams(vmem_limit_bytes=100 * 1024 * 1024),
    )(A_x.reshape(S, D).T, A_wqkv, A_wo, B_w_gate, B_w_up, B_w_down.T)
    return out.T.reshape(1, S, D)
```

```python
import numpy as np
import jax
import jax.numpy as jnp
from jax import lax
import jax.experimental.pallas as pl
import jax.experimental.pallas.tpu as pltpu

S, D, H, DH, W, DIL, DF = 2048, 576, 32, 18, 8, 2, 4608
DP = 640
NQ = 1792
R = 256
NB = S // R
FC = 1152
NC = DF // FC
NS = FC // 128
HALO = 16
f32, bf16 = jnp.float32, jnp.bfloat16
NT = (((1,), (1,)), ((), ()))
LW = (128, 128, 128, 128, 64)


def _gelu(g):
    c = np.float32(np.sqrt(2.0 / np.pi))
    return 0.5 * g * (1.0 + jnp.tanh(c * (g + np.float32(0.044715) * (g * g * g))))


def kernel(xT_hbm, wqkv_hbm, wo_hbm, wg_hbm, wu_hbm, wdT_hbm, outT_hbm,
           xio, xs, ost, wqkv_raw, wo_raw, wt, wall, woT, wg, wu, wdT,
           xn, xn_cur, xn_next, flag, x1b, q_s, k_s, v_s, o_s, h_s, acc, sems):
    SEM_X0, SEM_XR, SEM_WO, SEM_OUT, SEM_QKV, SEM_F = 0, 1, 2, 3, 4, 9
    cp_x0 = pltpu.make_async_copy(xT_hbm.at[:, pl.ds(0, R)], xio.at[:, pl.ds(0, R)], sems.at[SEM_X0])
    cp_xr = pltpu.make_async_copy(xT_hbm.at[:, pl.ds(R, S - R)], xio.at[:, pl.ds(R, S - R)], sems.at[SEM_XR])
    cp_wo = pltpu.make_async_copy(wo_hbm, wo_raw, sems.at[SEM_WO])

    def cp_qkv(lt):
        sl = pl.ds(lt * 128, LW[lt])
        return pltpu.make_async_copy(wqkv_hbm.at[sl, :], wqkv_raw.at[sl, :], sems.at[SEM_QKV + lt])

    def cp_ffn(c):
        sl = pl.ds(pl.multiple_of(c * FC, 128), FC)
        return [pltpu.make_async_copy(wg_hbm.at[:, sl], wg.at[pl.ds(0, D), sl], sems.at[SEM_F + 3 * c]),
                pltpu.make_async_copy(wu_hbm.at[:, sl], wu.at[pl.ds(0, D), sl], sems.at[SEM_F + 3 * c + 1]),
                pltpu.make_async_copy(wdT_hbm.at[:, sl], wdT.at[:, sl], sems.at[SEM_F + 3 * c + 2])]

    for lt in range(5):
        cp_qkv(lt).start()
    cp_x0.start()
    cp_wo.start()

    wg[D:DP, :] = jnp.zeros((DP - D, DF), bf16)
    wu[D:DP, :] = jnp.zeros((DP - D, DF), bf16)
    wall[:, 512:DP] = jnp.zeros((NQ, 128), bf16)
    wall[3 * D:NQ, 0:512] = jnp.zeros((NQ - 3 * D, 512), bf16)
    woT[:, 512:DP] = jnp.zeros((D, 128), bf16)
    for r_ in (xn, xn_cur, xn_next):
        r_[:, 512:DP] = jnp.zeros((R, 128), bf16)
    flag[...] = jnp.zeros(flag.shape, jnp.int32)
    k_s[:, 0:HALO, :] = jnp.zeros((5, HALO, 128), f32)
    v_s[:, 0:HALO, :] = jnp.zeros((5, HALO, 128), f32)
    xs[...] = jnp.zeros(xs.shape, f32)

    for lt in range(5):
        cp_qkv(lt).wait()
        if lt == 4:
            for cp in cp_ffn(0):
                cp.start()
            cp_xr.start()
        lw = LW[lt]
        wt[lt, :, 0:lw] = wqkv_raw[lt * 128:lt * 128 + lw, :].astype(f32).T
        for p in range(3):
            for d in range(DH):
                base = p * 512 + d * 32 if d < 16 else 1536 + p * 64 + (d - 16) * 32
                blk = wt[lt, pl.ds(p * D + d, H, stride=DH), :]
                wall[base:base + H, lt * 128:lt * 128 + lw] = blk[:, 0:lw].astype(bf16)
    cp_wo.wait()
    wof = wo_raw[...].astype(f32)
    for lt in range(5):
        wt[lt, 0:D, 0:LW[lt]] = wof[:, lt * 128:lt * 128 + LW[lt]]
    rows = [jnp.concatenate([wt[lt, pl.ds(d, H, stride=DH), :][:, 0:LW[lt]] for lt in range(5)], axis=1)
            for d in range(DH)]
    woT[:, 0:D] = jnp.concatenate(rows, axis=0).T.astype(bf16)
    for cp in cp_ffn(1):
        cp.start()

    scale = np.float32(DH ** -0.5)
    sub = lax.broadcasted_iota(jnp.int32, (8, 128), 0)

    def ln_to(xb, dst):
        m = jnp.sum(xb, axis=0, keepdims=True) * np.float32(1.0 / D)
        xc = xb - m
        v = jnp.sum(xc * xc, axis=0, keepdims=True) * np.float32(1.0 / D)
        xnt = xc * (1.0 / jnp.sqrt(v + 1e-5))
        dst[:, 0:D] = xnt.T.astype(bf16)

    def x_in(t):
        ca = pl.multiple_of((t % NB) * R, R)
        return jnp.where(t < NB, xio[:, pl.ds(ca, R)].astype(f32), xs[:, pl.ds(ca, R)])

    def stage_l1(t):
        ln_to(x_in(t), xn)

    def q_part(r0, n, part):
        xnv = xn[r0:r0 + n, :]
        rq, rk = slice(r0, r0 + n), slice(HALO + r0, HALO + r0 + n)
        if part == 3:
            tl = lax.dot_general(xnv, wall[1536:1792, :], NT, preferred_element_type=f32)
            lo = lax.broadcasted_iota(jnp.int32, (n, 128), 1) < 64
            t12 = tl[:, 0:128]
            q_s[rq, 512:640] = jnp.where(lo, t12, 0.0)
            k_s[4, rk, :] = jnp.where(lo, pltpu.roll(t12, 64, 1), 0.0)
            v_s[4, rk, :] = tl[:, 128:256]
            return tl[0:8, 0:128]
        r = lax.dot_general(xnv, wall[part * 512:(part + 1) * 512, :], NT, preferred_element_type=f32)
        if part == 0:
            q_s[rq, 0:512] = r
        else:
            dst = k_s if part == 1 else v_s
            for tt in range(4):
                dst[tt, rk, :] = r[:, tt * 128:(tt + 1) * 128]
        return r[0:8, 0:128]

    def t_slab(first, s0, tok=None):
        q = [q_s[s0:s0 + 8, tt * 128:(tt + 1) * 128] for tt in range(5)]
        if tok is not None:
            q = [x + tok for x in q]
        logits = []
        for w in range(W):
            off = HALO + s0 - w * DIL
            tsum = None
            for tt in range(5):
                pr = q[tt] * k_s[tt, off:off + 8, :]
                tsum = pr if tsum is None else tsum + pr
            tsum = tsum + pltpu.roll(tsum, 64, 1)
            tsum = tsum + pltpu.roll(tsum, 32, 1)
            tsum = tsum * scale
            if s0 < w * DIL:
                bad = jnp.logical_and(first, sub + s0 < w * DIL)
                tsum = jnp.where(bad, np.float32(-1e9), tsum)
            logits.append(tsum)
        m = logits[0]
        for w in range(1, W):
            m = jnp.maximum(m, logits[w])
        es = [jnp.exp(l - m) for l in logits]
        ssum = es[0]
        for w in range(1, W):
            ssum = ssum + es[w]
        inv = 1.0 / ssum
        for tt in range(5):
            o = None
            for w in range(W):
                off = HALO + s0 - w * DIL
                pv = es[w] * v_s[tt, off:off + 8, :]
                o = pv if o is None else o + pv
            o_s[s0:s0 + 8, tt * 128:(tt + 1) * 128] = o * inv

    def dot_nt_rows(lhs_ref, cols, rhs, nsplit):
        rs = D // nsplit
        return jnp.concatenate(
            [lax.dot_general(lhs_ref[i * rs:(i + 1) * rs, cols], rhs, NT, preferred_element_type=f32)
             for i in range(nsplit)], axis=0)

    def halo_roll():
        k_s[:, 0:HALO, :] = k_s[:, R:R + HALO, :]
        v_s[:, 0:HALO, :] = v_s[:, R:R + HALO, :]

    def stage_o(t):
        y = dot_nt_rows(woT, slice(0, DP), o_s[...].astype(bf16), 3)
        x1b[...] = x_in(t) + y
        halo_roll()

    def f_gu(f0, n):
        xnv = xn_cur[...]
        g = jnp.dot(xnv, wg[:, pl.ds(f0, n)], preferred_element_type=f32)
        u = jnp.dot(xnv, wu[:, pl.ds(f0, n)], preferred_element_type=f32)
        return g, (_gelu(g) * u).astype(bf16)

    def f_sub(c, sb):
        g, h = f_gu(c * FC + sb * 128, 128)
        h_s[c % 2, :, sb * 128:(sb + 1) * 128] = h
        return g[0:8, :]

    def f_down(c):
        src = x1b if c == 0 else acc
        acc[...] = src[...] + dot_nt_rows(wdT, slice(c * FC, (c + 1) * FC), h_s[c % 2], 2)

    def out_block(b):
        cb = pl.multiple_of(b * R, R)
        ost[:, pl.ds(cb, R)] = xs[:, pl.ds(cb, R)].astype(bf16)
        pltpu.make_async_copy(ost.at[:, pl.ds(cb, R)], outT_hbm.at[:, pl.ds(cb, R)], sems.at[SEM_OUT]).start()

    def a_only(t):
        first = t % NB == 0
        never = flag[...] != 0
        stage_l1(t)
        for part in (3, 1, 2, 0):
            q_part(0, 128, part)
        for i, part in enumerate((3, 1, 2, 0)):
            tok = jnp.where(never, q_part(128, 128, part), 0.0)
            for j in range(4):
                t_slab(first, 8 * (4 * i + j), tok)
        xin = x_in(t)
        for hh in range(2):
            ls = slice(hh * 128, (hh + 1) * 128)
            if hh == 1:
                for s0 in range(128, R, 8):
                    t_slab(first, s0)
            x1 = xin[:, ls] + dot_nt_rows(woT, slice(0, DP), o_s[ls, :].astype(bf16), 3)
            x1b[:, ls] = x1
            ln_to(x1, xn_cur.at[pl.ds(hh * 128, 128)])
        halo_roll()

    def slot(t, carry):
        never = flag[...] != 0
        first = (t + 1) % NB == 0
        extra = {}

        def at(i, fn):
            extra.setdefault(i, []).append(fn)
        at(0, lambda tok: stage_l1(t + 1))
        at(3, lambda tok: [q_part(0, R, part) for part in (0, 1, 2, 3)])
        pos = list(range(8, 24))
        for i in range(R // 8):
            at(pos[(i * len(pos)) // (R // 8)], lambda tok, i=i: t_slab(first, 8 * i, tok))
        at(25, lambda tok: stage_o(t + 1))
        at(27, lambda tok: ln_to(x1b[...], xn_next))
        for c in range(NC):
            for sb in range(NS):
                dep = f_sub(c, sb)
                if c > 0 and sb == 1:
                    f_down(c - 1)
                i = c * NS + sb
                if i in extra:
                    tok = jnp.where(never, dep, 0.0)
                    for p in extra[i]:
                        p(tok)
        xn_cur[...] = xn_next[...]
        f_down(NC - 1)
        xs[:, pl.ds(pl.multiple_of((t % NB) * R, R), R)] = acc[...]

        @pl.when(t >= NB)
        def _():
            out_block(t % NB)
        return carry

    def f_only(t, first_pass):
        acc[...] = x1b[...]

        def cbody(c, carry):
            @pl.when(first_pass)
            def _():
                for cp in cp_ffn(c):
                    cp.wait()
            f0 = pl.multiple_of(c * FC, FC)
            _, h = f_gu(f0, FC)
            acc[...] += lax.dot_general(wdT[:, pl.ds(f0, FC)], h, NT, preferred_element_type=f32)
            return carry

        lax.fori_loop(0, NC, cbody, 0)
        xs[:, pl.ds(pl.multiple_of((t % NB) * R, R), R)] = acc[...]

    cp_x0.wait()

    def pass_body(p, carry):
        @pl.when(p == 1)
        def _():
            cp_xr.wait()

        a_only(p)

        @pl.when(p == 0)
        def _():
            for c in range(2, NC):
                for cp in cp_ffn(c):
                    cp.start()

        @pl.when(p == 1)
        def _():
            lax.fori_loop(1, 2 * NB - 1, slot, 0)

        f_only(p * (2 * NB - 1), p == 0)
        return carry

    lax.fori_loop(0, 2, pass_body, 0)
    out_block(NB - 1)
    pltpu.make_async_copy(ost, outT_hbm, sems.at[SEM_OUT]).wait()


@jax.jit
def pallas_interleave_layers__sliding_local_dilated__glu_gated_geglu__prompt_kernel(
        A_x, A_wqkv, A_wo, B_x, B_w_gate, B_w_up, B_w_down):
    hbm = pl.BlockSpec(memory_space=pltpu.HBM)
    out = pl.pallas_call(
        kernel,
        out_shape=jax.ShapeDtypeStruct((D, S), bf16),
        in_specs=[hbm] * 6,
        out_specs=hbm,
        scratch_shapes=[
            pltpu.VMEM((D, S), bf16),
            pltpu.VMEM((D, S), f32),
            pltpu.VMEM((D, S), bf16),
            pltpu.VMEM((D, 3 * D), bf16),
            pltpu.VMEM((D, D), bf16),
            pltpu.VMEM((5, 3 * D, 128), f32),
            pltpu.VMEM((NQ, DP), bf16),
            pltpu.VMEM((D, DP), bf16),
            pltpu.VMEM((DP, DF), bf16),
            pltpu.VMEM((DP, DF), bf16),
            pltpu.VMEM((D, DF), bf16),
            pltpu.VMEM((R, DP), bf16),
            pltpu.VMEM((R, DP), bf16),
            pltpu.VMEM((R, DP), bf16),
            pltpu.VMEM((8, 128), jnp.int32),
            pltpu.VMEM((D, R), f32),
            pltpu.VMEM((R, DP), f32),
            pltpu.VMEM((5, HALO + R, 128), f32),
            pltpu.VMEM((5, HALO + R, 128), f32),
            pltpu.VMEM((R, DP), f32),
            pltpu.VMEM((2, R, FC), bf16),
            pltpu.VMEM((D, R), f32),
            pltpu.SemaphoreType.DMA((9 + 3 * NC,)),
        ],
        compiler_params=pltpu.CompilerParams(vmem_limit_bytes=100 * 1024 * 1024),
    )(A_x.reshape(S, D).T, A_wqkv, A_wo, B_w_gate, B_w_up, B_w_down.T)
    return out.T.reshape(1, S, D)
```

```python
import numpy as np
import jax
import jax.numpy as jnp
from jax import lax
import jax.experimental.pallas as pl
import jax.experimental.pallas.tpu as pltpu

S, D, H, DH, W, DIL, DF = 2048, 576, 32, 18, 8, 2, 4608
DP = 640
NQ = 1792
R = 256
NB = S // R
FC = 1152
NC = DF // FC
NS = FC // 128
HALO = 16
f32, bf16 = jnp.float32, jnp.bfloat16
NT = (((1,), (1,)), ((), ()))
LW = (128, 128, 128, 128, 64)


def _gelu(g):
    c = np.float32(np.sqrt(2.0 / np.pi))
    return 0.5 * g * (1.0 + jnp.tanh(c * (g + np.float32(0.044715) * (g * g * g))))


def kernel(xT_hbm, wqkv_hbm, wo_hbm, wg_hbm, wu_hbm, wdT_hbm, outT_hbm,
           xio, xs, ost, wqkv_raw, wo_raw, wt, wall, woT, wg, wu, wdT,
           xn, xn_cur, flag, x1b, q_s, k_s, v_s, o_s, h_s, acc, sems):
    SEM_X0, SEM_XR, SEM_WO, SEM_OUT, SEM_QKV, SEM_F = 0, 1, 2, 3, 4, 9
    cp_x0 = pltpu.make_async_copy(xT_hbm.at[:, pl.ds(0, R)], xio.at[:, pl.ds(0, R)], sems.at[SEM_X0])
    cp_xr = pltpu.make_async_copy(xT_hbm.at[:, pl.ds(R, S - R)], xio.at[:, pl.ds(R, S - R)], sems.at[SEM_XR])
    cp_wo = pltpu.make_async_copy(wo_hbm, wo_raw, sems.at[SEM_WO])

    def cp_qkv(lt):
        sl = pl.ds(lt * 128, LW[lt])
        return pltpu.make_async_copy(wqkv_hbm.at[sl, :], wqkv_raw.at[sl, :], sems.at[SEM_QKV + lt])

    def cp_ffn(c, i):
        sl = pl.ds(pl.multiple_of(c * FC, 128), FC)
        src, dst = ((wg_hbm, wg), (wu_hbm, wu), (wdT_hbm, wdT))[i]
        return pltpu.make_async_copy(src.at[:, sl], dst.at[pl.ds(0, D), sl], sems.at[SEM_F + 3 * c + i])

    for lt in range(5):
        cp_qkv(lt).start()
    cp_x0.start()
    cp_wo.start()

    wg[D:DP, :] = jnp.zeros((DP - D, DF), bf16)
    wu[D:DP, :] = jnp.zeros((DP - D, DF), bf16)
    wall[:, 512:DP] = jnp.zeros((NQ, 128), bf16)
    wall[3 * D:NQ, 0:512] = jnp.zeros((NQ - 3 * D, 512), bf16)
    woT[:, 512:DP] = jnp.zeros((D, 128), bf16)
    for r_ in (xn, xn_cur):
        r_[:, 512:DP] = jnp.zeros((R, 128), bf16)
    flag[...] = jnp.zeros(flag.shape, jnp.int32)
    k_s[:, 0:HALO, :] = jnp.zeros((5, HALO, 128), f32)
    v_s[:, 0:HALO, :] = jnp.zeros((5, HALO, 128), f32)
    xs[...] = jnp.zeros(xs.shape, f32)

    for lt in range(5):
        cp_qkv(lt).wait()
        if lt == 4:
            for i in range(3):
                cp_ffn(0, i).start()
        lw = LW[lt]
        wt[lt, :, 0:lw] = wqkv_raw[lt * 128:lt * 128 + lw, :].astype(f32).T
        for p in range(3):
            for d in range(DH):
                base = p * 512 + d * 32 if d < 16 else 1536 + p * 64 + (d - 16) * 32
                blk = wt[lt, pl.ds(p * D + d, H, stride=DH), :]
                wall[base:base + H, lt * 128:lt * 128 + lw] = blk[:, 0:lw].astype(bf16)
    cp_ffn(1, 0).start()

    def prep_wo():
        wof = wo_raw[...].astype(f32)
        for lt in range(5):
            wt[lt, 0:D, 0:LW[lt]] = wof[:, lt * 128:lt * 128 + LW[lt]]
        rows = [jnp.concatenate([wt[lt, pl.ds(d, H, stride=DH), :][:, 0:LW[lt]] for lt in range(5)], axis=1)
                for d in range(DH)]
        woT[:, 0:D] = jnp.concatenate(rows, axis=0).T.astype(bf16)

    scale = np.float32(DH ** -0.5)
    sub = lax.broadcasted_iota(jnp.int32, (8, 128), 0)

    def ln_to(xb, dst):
        m = jnp.sum(xb, axis=0, keepdims=True) * np.float32(1.0 / D)
        xc = xb - m
        v = jnp.sum(xc * xc, axis=0, keepdims=True) * np.float32(1.0 / D)
        xnt = xc * (1.0 / jnp.sqrt(v + 1e-5))
        dst[:, 0:D] = xnt.T.astype(bf16)

    def x_in(t):
        ca = pl.multiple_of((t % NB) * R, R)
        return jnp.where(t < NB, xio[:, pl.ds(ca, R)].astype(f32), xs[:, pl.ds(ca, R)])

    def stage_l1(t):
        ln_to(x_in(t), xn)

    def q_part(r0, n, part):
        xnv = xn[r0:r0 + n, :]
        rq, rk = slice(r0, r0 + n), slice(HALO + r0, HALO + r0 + n)
        if part == 3:
            tl = lax.dot_general(xnv, wall[1536:1792, :], NT, preferred_element_type=f32)
            lo = lax.broadcasted_iota(jnp.int32, (n, 128), 1) < 64
            t12 = tl[:, 0:128]
            q_s[rq, 512:640] = jnp.where(lo, t12, 0.0)
            k_s[4, rk, :] = jnp.where(lo, pltpu.roll(t12, 64, 1), 0.0)
            v_s[4, rk, :] = tl[:, 128:256]
            return tl[0:8, 0:128]
        r = lax.dot_general(xnv, wall[part * 512:(part + 1) * 512, :], NT, preferred_element_type=f32)
        if part == 0:
            q_s[rq, 0:512] = r
        else:
            dst = k_s if part == 1 else v_s
            for tt in range(4):
                dst[tt, rk, :] = r[:, tt * 128:(tt + 1) * 128]
        return r[0:8, 0:128]

    def t_slab(first, s0, tok=None):
        q = [q_s[s0:s0 + 8, tt * 128:(tt + 1) * 128] for tt in range(5)]
        if tok is not None:
            q = [x + tok for x in q]
        logits = []
        for w in range(W):
            off = HALO + s0 - w * DIL
            tsum = None
            for tt in range(5):
                pr = q[tt] * k_s[tt, off:off + 8, :]
                tsum = pr if tsum is None else tsum + pr
            tsum = tsum + pltpu.roll(tsum, 64, 1)
            tsum = tsum + pltpu.roll(tsum, 32, 1)
            tsum = tsum * scale
            if s0 < w * DIL:
                bad = jnp.logical_and(first, sub + s0 < w * DIL)
                tsum = jnp.where(bad, np.float32(-1e9), tsum)
            logits.append(tsum)
        m = logits[0]
        for w in range(1, W):
            m = jnp.maximum(m, logits[w])
        es = [jnp.exp(l - m) for l in logits]
        ssum = es[0]
        for w in range(1, W):
            ssum = ssum + es[w]
        inv = 1.0 / ssum
        for tt in range(5):
            o = None
            for w in range(W):
                off = HALO + s0 - w * DIL
                pv = es[w] * v_s[tt, off:off + 8, :]
                o = pv if o is None else o + pv
            o_s[s0:s0 + 8, tt * 128:(tt + 1) * 128] = o * inv

    def dot_nt_rows(lhs_ref, cols, rhs, nsplit):
        rs = D // nsplit
        return jnp.concatenate(
            [lax.dot_general(lhs_ref[i * rs:(i + 1) * rs, cols], rhs, NT, preferred_element_type=f32)
             for i in range(nsplit)], axis=0)

    def halo_roll():
        k_s[:, 0:HALO, :] = k_s[:, R:R + HALO, :]
        v_s[:, 0:HALO, :] = v_s[:, R:R + HALO, :]

    def stage_o(t):
        y = dot_nt_rows(woT, slice(0, DP), o_s[...].astype(bf16), 3)
        x1b[...] = x_in(t) + y
        halo_roll()

    def f_gu(f0, n):
        xnv = xn_cur[...]
        g = jnp.dot(xnv, wg[:, pl.ds(f0, n)], preferred_element_type=f32)
        u = jnp.dot(xnv, wu[:, pl.ds(f0, n)], preferred_element_type=f32)
        return g, (_gelu(g) * u).astype(bf16)

    def f_sub(c, sb):
        g, h = f_gu(c * FC + sb * 128, 128)
        h_s[c % 2, :, sb * 128:(sb + 1) * 128] = h
        return g[0:8, :]

    def f_down(c, store=True):
        src = x1b if c == 0 else acc
        r = src[...] + dot_nt_rows(wdT, slice(c * FC, (c + 1) * FC), h_s[c % 2], 3)
        if store:
            acc[...] = r
        return r

    def out_dma(b):
        cb = pl.multiple_of(b * R, R)
        return pltpu.make_async_copy(ost.at[:, pl.ds(cb, R)], outT_hbm.at[:, pl.ds(cb, R)], sems.at[SEM_OUT])

    def a_only(t):
        first = t % NB == 0
        never = flag[...] != 0
        stage_l1(t)
        for part in (3, 1, 2, 0):
            q_part(0, 128, part)
        prep_wo()
        for i, part in enumerate((3, 1, 2, 0)):
            tok = jnp.where(never, q_part(128, 128, part), 0.0)
            for j in range(4):
                t_slab(first, 8 * (4 * i + j), tok)
        xin = x_in(t)
        for hh in range(2):
            ls = slice(hh * 128, (hh + 1) * 128)
            if hh == 1:
                for s0 in range(128, R, 8):
                    t_slab(first, s0)
            x1 = xin[:, ls] + dot_nt_rows(woT, slice(0, DP), o_s[ls, :].astype(bf16), 3)
            x1b[:, ls] = x1
            ln_to(x1, xn_cur.at[pl.ds(hh * 128, 128)])
        halo_roll()

    def slot(t, carry):
        never = flag[...] != 0
        first = (t + 1) % NB == 0
        extra = {}

        def at(i, fn):
            extra.setdefault(i, []).append(fn)
        at(1, lambda tok: stage_l1(t + 1))
        at(2, lambda tok: [q_part(0, R, part) for part in (2, 3, 1, 0)])
        pos = list(range(7, 25))
        for i in range(R // 8):
            at(pos[(i * len(pos)) // (R // 8)], lambda tok, i=i: t_slab(first, 8 * i, tok))
        at(25, lambda tok: stage_o(t + 1))
        for c in range(NC):
            for sb in range(NS):
                dep = f_sub(c, sb)
                if c > 0 and sb == 0:
                    f_down(c - 1)
                i = c * NS + sb
                if i in extra:
                    tok = jnp.where(never, dep, 0.0)
                    for p in extra[i]:
                        p(tok)
        ln_to(x1b[...], xn_cur)
        cb = pl.multiple_of((t % NB) * R, R)
        r = f_down(NC - 1, store=False)
        xs[:, pl.ds(cb, R)] = r
        ost[:, pl.ds(cb, R)] = r.astype(bf16)

        @pl.when(t >= NB)
        def _():
            out_dma(t % NB).start()
        return carry

    def f_only(t, first_pass):
        acc[...] = x1b[...]

        def cbody(c, carry):
            @pl.when(first_pass)
            def _():
                for i in range(3):
                    cp_ffn(c, i).wait()
                for cs in range(1, NC - 1):
                    @pl.when(c == cs)
                    def _():
                        cp_ffn(cs + 1, 1).start()
                        cp_ffn(cs + 1, 2).start()
                        if cs + 2 < NC:
                            cp_ffn(cs + 2, 0).start()
                        else:
                            cp_xr.start()
            f0 = pl.multiple_of(c * FC, FC)
            _, h = f_gu(f0, FC)
            acc[...] += lax.dot_general(wdT[:, pl.ds(f0, FC)], h, NT, preferred_element_type=f32)
            return carry

        lax.fori_loop(0, NC, cbody, 0)
        xs[:, pl.ds(pl.multiple_of((t % NB) * R, R), R)] = acc[...]

    cp_x0.wait()
    cp_wo.wait()

    def pass_body(p, carry):
        @pl.when(p == 1)
        def _():
            cp_xr.wait()

        a_only(p)

        @pl.when(p == 0)
        def _():
            cp_ffn(1, 1).start()
            cp_ffn(1, 2).start()
            cp_ffn(2, 0).start()

        @pl.when(p == 1)
        def _():
            lax.fori_loop(1, 2 * NB - 1, slot, 0)

        f_only(p * (2 * NB - 1), p == 0)
        return carry

    lax.fori_loop(0, 2, pass_body, 0)
    ost[:, S - R:S] = xs[:, S - R:S].astype(bf16)
    out_dma(NB - 1).start()
    pltpu.make_async_copy(ost, outT_hbm, sems.at[SEM_OUT]).wait()


@jax.jit
def pallas_interleave_layers__sliding_local_dilated__glu_gated_geglu__prompt_kernel(
        A_x, A_wqkv, A_wo, B_x, B_w_gate, B_w_up, B_w_down):
    hbm = pl.BlockSpec(memory_space=pltpu.HBM)
    out = pl.pallas_call(
        kernel,
        out_shape=jax.ShapeDtypeStruct((D, S), bf16),
        in_specs=[hbm] * 6,
        out_specs=hbm,
        scratch_shapes=[
            pltpu.VMEM((D, S), bf16),
            pltpu.VMEM((D, S), f32),
            pltpu.VMEM((D, S), bf16),
            pltpu.VMEM((D, 3 * D), bf16),
            pltpu.VMEM((D, D), bf16),
            pltpu.VMEM((5, 3 * D, 128), f32),
            pltpu.VMEM((NQ, DP), bf16),
            pltpu.VMEM((D, DP), bf16),
            pltpu.VMEM((DP, DF), bf16),
            pltpu.VMEM((DP, DF), bf16),
            pltpu.VMEM((D, DF), bf16),
            pltpu.VMEM((R, DP), bf16),
            pltpu.VMEM((R, DP), bf16),
            pltpu.VMEM((8, 128), jnp.int32),
            pltpu.VMEM((D, R), f32),
            pltpu.VMEM((R, DP), f32),
            pltpu.VMEM((5, HALO + R, 128), f32),
            pltpu.VMEM((5, HALO + R, 128), f32),
            pltpu.VMEM((R, DP), f32),
            pltpu.VMEM((2, R, FC), bf16),
            pltpu.VMEM((D, R), f32),
            pltpu.SemaphoreType.DMA((9 + 3 * NC,)),
        ],
        compiler_params=pltpu.CompilerParams(vmem_limit_bytes=100 * 1024 * 1024),
    )(A_x.reshape(S, D).T, A_wqkv, A_wo, B_w_gate, B_w_up, B_w_down.T)
    return out.T.reshape(1, S, D)
```

```python
import numpy as np
import jax
import jax.numpy as jnp
from jax import lax
import jax.experimental.pallas as pl
import jax.experimental.pallas.tpu as pltpu

S, D, H, DH, W, DIL, DF = 2048, 576, 32, 18, 8, 2, 4608
DP = 640
NQ = 1792
R = 256
NB = S // R
FC = 1152
NC = DF // FC
NS = FC // 128
HALO = 16
f32, bf16 = jnp.float32, jnp.bfloat16
NT = (((1,), (1,)), ((), ()))
LW = (128, 128, 128, 128, 64)


def _gelu(g):
    c = np.float32(np.sqrt(2.0 / np.pi))
    return 0.5 * g * (1.0 + jnp.tanh(c * (g + np.float32(0.044715) * (g * g * g))))


def kernel(xT_hbm, wqkv_hbm, wo_hbm, wg_hbm, wu_hbm, wdT_hbm, outT_hbm,
           xio, xs, ost, wqkv_raw, wo_raw, wt, wall, woT, wg, wu, wdT,
           xn, xn_cur, flag, x1b, q_s, k_s, v_s, o_s, h_s, acc, sems):
    SEM_X0, SEM_XR, SEM_WO, SEM_OUT, SEM_QKV, SEM_F = 0, 1, 2, 3, 4, 9
    cp_x0 = pltpu.make_async_copy(xT_hbm.at[:, pl.ds(0, R)], xio.at[:, pl.ds(0, R)], sems.at[SEM_X0])
    cp_xr = pltpu.make_async_copy(xT_hbm.at[:, pl.ds(R, S - R)], xio.at[:, pl.ds(R, S - R)], sems.at[SEM_XR])
    cp_wo = pltpu.make_async_copy(wo_hbm, wo_raw, sems.at[SEM_WO])

    def cp_qkv(lt):
        sl = pl.ds(lt * 128, LW[lt])
        return pltpu.make_async_copy(wqkv_hbm.at[sl, :], wqkv_raw.at[sl, :], sems.at[SEM_QKV + lt])

    def cp_ffn(c, i):
        sl = pl.ds(pl.multiple_of(c * FC, 128), FC)
        src, dst = ((wg_hbm, wg), (wu_hbm, wu), (wdT_hbm, wdT))[i]
        return pltpu.make_async_copy(src.at[:, sl], dst.at[pl.ds(0, D), sl], sems.at[SEM_F + 3 * c + i])

    for lt in range(5):
        cp_qkv(lt).start()
    cp_x0.start()
    cp_wo.start()

    wg[D:DP, :] = jnp.zeros((DP - D, DF), bf16)
    wu[D:DP, :] = jnp.zeros((DP - D, DF), bf16)
    wall[:, 512:DP] = jnp.zeros((NQ, 128), bf16)
    wall[3 * D:NQ, 0:512] = jnp.zeros((NQ - 3 * D, 512), bf16)
    woT[:, 512:DP] = jnp.zeros((D, 128), bf16)
    for r_ in (xn, xn_cur):
        r_[:, 512:DP] = jnp.zeros((R, 128), bf16)
    flag[...] = jnp.zeros(flag.shape, jnp.int32)
    k_s[:, 0:HALO, :] = jnp.zeros((5, HALO, 128), f32)
    v_s[:, 0:HALO, :] = jnp.zeros((5, HALO, 128), f32)
    xs[...] = jnp.zeros(xs.shape, f32)

    for lt in range(5):
        cp_qkv(lt).wait()
        if lt == 4:
            for i in range(3):
                cp_ffn(0, i).start()
        lw = LW[lt]
        wt[lt, :, 0:lw] = wqkv_raw[lt * 128:lt * 128 + lw, :].astype(f32).T
        for p in range(3):
            for d in range(DH):
                base = p * 512 + d * 32 if d < 16 else 1536 + p * 64 + (d - 16) * 32
                blk = wt[lt, pl.ds(p * D + d, H, stride=DH), :]
                wall[base:base + H, lt * 128:lt * 128 + lw] = blk[:, 0:lw].astype(bf16)
    cp_ffn(1, 0).start()

    def prep_wo():
        wof = wo_raw[...].astype(f32)
        for lt in range(5):
            wt[lt, 0:D, 0:LW[lt]] = wof[:, lt * 128:lt * 128 + LW[lt]]
        rows = [jnp.concatenate([wt[lt, pl.ds(d, H, stride=DH), :][:, 0:LW[lt]] for lt in range(5)], axis=1)
                for d in range(DH)]
        woT[:, 0:D] = jnp.concatenate(rows, axis=0).T.astype(bf16)

    scale = np.float32(DH ** -0.5)
    sub = lax.broadcasted_iota(jnp.int32, (8, 128), 0)

    def ln_to(xb, dst):
        m = jnp.sum(xb, axis=0, keepdims=True) * np.float32(1.0 / D)
        xc = xb - m
        v = jnp.sum(xc * xc, axis=0, keepdims=True) * np.float32(1.0 / D)
        xnt = xc * (1.0 / jnp.sqrt(v + 1e-5))
        dst[:, 0:D] = xnt.T.astype(bf16)

    def x_in(t):
        ca = pl.multiple_of((t % NB) * R, R)
        return jnp.where(t < NB, xio[:, pl.ds(ca, R)].astype(f32), xs[:, pl.ds(ca, R)])

    def stage_l1(t):
        ln_to(x_in(t), xn)

    def q_part(r0, n, part):
        xnv = xn[r0:r0 + n, :]
        rq, rk = slice(r0, r0 + n), slice(HALO + r0, HALO + r0 + n)
        if part == 3:
            tl = lax.dot_general(xnv, wall[1536:1792, :], NT, preferred_element_type=f32)
            lo = lax.broadcasted_iota(jnp.int32, (n, 128), 1) < 64
            t12 = tl[:, 0:128]
            q_s[rq, 512:640] = jnp.where(lo, t12, 0.0)
            k_s[4, rk, :] = jnp.where(lo, pltpu.roll(t12, 64, 1), 0.0)
            v_s[4, rk, :] = tl[:, 128:256]
            return tl[0:8, 0:128]
        r = lax.dot_general(xnv, wall[part * 512:(part + 1) * 512, :], NT, preferred_element_type=f32)
        if part == 0:
            q_s[rq, 0:512] = r
        else:
            dst = k_s if part == 1 else v_s
            for tt in range(4):
                dst[tt, rk, :] = r[:, tt * 128:(tt + 1) * 128]
        return r[0:8, 0:128]

    def t_slab(first, s0, tok=None):
        q = [q_s[s0:s0 + 8, tt * 128:(tt + 1) * 128] for tt in range(5)]
        if tok is not None:
            q = [x + tok for x in q]
        logits = []
        for w in range(W):
            off = HALO + s0 - w * DIL
            tsum = None
            for tt in range(5):
                pr = q[tt] * k_s[tt, off:off + 8, :]
                tsum = pr if tsum is None else tsum + pr
            tsum = tsum + pltpu.roll(tsum, 64, 1)
            tsum = tsum + pltpu.roll(tsum, 32, 1)
            tsum = tsum * scale
            if s0 < w * DIL:
                bad = jnp.logical_and(first, sub + s0 < w * DIL)
                tsum = jnp.where(bad, np.float32(-1e9), tsum)
            logits.append(tsum)
        m = logits[0]
        for w in range(1, W):
            m = jnp.maximum(m, logits[w])
        es = [jnp.exp(l - m) for l in logits]
        ssum = es[0]
        for w in range(1, W):
            ssum = ssum + es[w]
        inv = 1.0 / ssum
        for tt in range(5):
            o = None
            for w in range(W):
                off = HALO + s0 - w * DIL
                pv = es[w] * v_s[tt, off:off + 8, :]
                o = pv if o is None else o + pv
            o_s[s0:s0 + 8, tt * 128:(tt + 1) * 128] = o * inv

    def dot_nt_rows(lhs_ref, cols, rhs, nsplit):
        rs = D // nsplit
        return jnp.concatenate(
            [lax.dot_general(lhs_ref[i * rs:(i + 1) * rs, cols], rhs, NT, preferred_element_type=f32)
             for i in range(nsplit)], axis=0)

    def halo_roll():
        k_s[:, 0:HALO, :] = k_s[:, R:R + HALO, :]
        v_s[:, 0:HALO, :] = v_s[:, R:R + HALO, :]

    def stage_o(t):
        y = dot_nt_rows(woT, slice(0, DP), o_s[...].astype(bf16), 3)
        x1b[...] = x_in(t) + y
        halo_roll()

    def f_gu(f0, n):
        xnv = xn_cur[...]
        g = jnp.dot(xnv, wg[:, pl.ds(f0, n)], preferred_element_type=f32)
        u = jnp.dot(xnv, wu[:, pl.ds(f0, n)], preferred_element_type=f32)
        return g, (_gelu(g) * u).astype(bf16)

    def f_sub(c, sb):
        g, h = f_gu(c * FC + sb * 128, 128)
        h_s[c % 2, :, sb * 128:(sb + 1) * 128] = h
        return g[0:8, :]

    def f_down(c, store=True):
        src = x1b if c == 0 else acc
        r = src[...] + dot_nt_rows(wdT, slice(c * FC, (c + 1) * FC), h_s[c % 2], 3)
        if store:
            acc[...] = r
        return r

    def out_dma(b):
        cb = pl.multiple_of(b * R, R)
        return pltpu.make_async_copy(ost.at[:, pl.ds(cb, R)], outT_hbm.at[:, pl.ds(cb, R)], sems.at[SEM_OUT])

    def a_only(t):
        first = t % NB == 0
        never = flag[...] != 0
        stage_l1(t)
        for part in (1, 3, 0):
            q_part(0, 128, part)
        prep_wo()
        q_part(0, 128, 2)
        s0 = 0
        for part, cnt in ((3, 5), (1, 4), (0, 4), (2, 3)):
            tok = jnp.where(never, q_part(128, 128, part), 0.0)
            for _ in range(cnt):
                t_slab(first, s0, tok)
                s0 += 8
        xin = x_in(t)
        for hh in range(2):
            ls = slice(hh * 128, (hh + 1) * 128)
            if hh == 1:
                for s0 in range(128, R, 8):
                    t_slab(first, s0)
            x1 = xin[:, ls] + dot_nt_rows(woT, slice(0, DP), o_s[ls, :].astype(bf16), 6)
            x1b[:, ls] = x1
            ln_to(x1, xn_cur.at[pl.ds(hh * 128, 128)])
        halo_roll()

    def slot(t, carry):
        never = flag[...] != 0
        first = (t + 1) % NB == 0
        extra = {}

        def at(i, fn):
            extra.setdefault(i, []).append(fn)
        at(1, lambda tok: stage_l1(t + 1))
        at(2, lambda tok: [q_part(0, R, part) for part in (2, 3, 1, 0)])
        pos = list(range(7, 25))
        for i in range(R // 8):
            at(pos[(i * len(pos)) // (R // 8)], lambda tok, i=i: t_slab(first, 8 * i, tok))
        at(25, lambda tok: stage_o(t + 1))
        for c in range(NC):
            for sb in range(NS):
                dep = f_sub(c, sb)
                if c > 0 and sb == 0:
                    f_down(c - 1)
                i = c * NS + sb
                if i in extra:
                    tok = jnp.where(never, dep, 0.0)
                    for p in extra[i]:
                        p(tok)
        ln_to(x1b[...], xn_cur)
        cb = pl.multiple_of((t % NB) * R, R)
        r = f_down(NC - 1, store=False)
        xs[:, pl.ds(cb, R)] = r
        ost[:, pl.ds(cb, R)] = r.astype(bf16)

        @pl.when(t >= NB)
        def _():
            out_dma(t % NB).start()
        return carry

    def f_only(t, first_pass):
        acc[...] = x1b[...]

        def cbody(c, carry):
            @pl.when(first_pass)
            def _():
                for i in range(3):
                    cp_ffn(c, i).wait()
                for cs in range(1, NC - 1):
                    @pl.when(c == cs)
                    def _():
                        cp_ffn(cs + 1, 1).start()
                        cp_ffn(cs + 1, 2).start()
                        if cs + 2 < NC:
                            cp_ffn(cs + 2, 0).start()
                        else:
                            cp_xr.start()
            f0 = pl.multiple_of(c * FC, FC)
            _, h = f_gu(f0, FC)
            acc[...] += lax.dot_general(wdT[:, pl.ds(f0, FC)], h, NT, preferred_element_type=f32)
            return carry

        lax.fori_loop(0, NC, cbody, 0)
        xs[:, pl.ds(pl.multiple_of((t % NB) * R, R), R)] = acc[...]

    cp_x0.wait()
    cp_wo.wait()

    def pass_body(p, carry):
        @pl.when(p == 1)
        def _():
            cp_xr.wait()

        a_only(p)

        @pl.when(p == 0)
        def _():
            cp_ffn(1, 1).start()
            cp_ffn(1, 2).start()
            cp_ffn(2, 0).start()

        @pl.when(p == 1)
        def _():
            lax.fori_loop(1, 2 * NB - 1, slot, 0)

        f_only(p * (2 * NB - 1), p == 0)
        return carry

    lax.fori_loop(0, 2, pass_body, 0)
    ost[:, S - R:S] = xs[:, S - R:S].astype(bf16)
    out_dma(NB - 1).start()
    pltpu.make_async_copy(ost, outT_hbm, sems.at[SEM_OUT]).wait()


@jax.jit
def pallas_interleave_layers__sliding_local_dilated__glu_gated_geglu__prompt_kernel(
        A_x, A_wqkv, A_wo, B_x, B_w_gate, B_w_up, B_w_down):
    hbm = pl.BlockSpec(memory_space=pltpu.HBM)
    out = pl.pallas_call(
        kernel,
        out_shape=jax.ShapeDtypeStruct((D, S), bf16),
        in_specs=[hbm] * 6,
        out_specs=hbm,
        scratch_shapes=[
            pltpu.VMEM((D, S), bf16),
            pltpu.VMEM((D, S), f32),
            pltpu.VMEM((D, S), bf16),
            pltpu.VMEM((D, 3 * D), bf16),
            pltpu.VMEM((D, D), bf16),
            pltpu.VMEM((5, 3 * D, 128), f32),
            pltpu.VMEM((NQ, DP), bf16),
            pltpu.VMEM((D, DP), bf16),
            pltpu.VMEM((DP, DF), bf16),
            pltpu.VMEM((DP, DF), bf16),
            pltpu.VMEM((D, DF), bf16),
            pltpu.VMEM((R, DP), bf16),
            pltpu.VMEM((R, DP), bf16),
            pltpu.VMEM((8, 128), jnp.int32),
            pltpu.VMEM((D, R), f32),
            pltpu.VMEM((R, DP), f32),
            pltpu.VMEM((5, HALO + R, 128), f32),
            pltpu.VMEM((5, HALO + R, 128), f32),
            pltpu.VMEM((R, DP), f32),
            pltpu.VMEM((2, R, FC), bf16),
            pltpu.VMEM((D, R), f32),
            pltpu.SemaphoreType.DMA((9 + 3 * NC,)),
        ],
        compiler_params=pltpu.CompilerParams(vmem_limit_bytes=100 * 1024 * 1024),
    )(A_x.reshape(S, D).T, A_wqkv, A_wo, B_w_gate, B_w_up, B_w_down.T)
    return out.T.reshape(1, S, D)
```
